```python
import os as _os
_os.environ.setdefault("JAX_PLATFORMS", "cpu")
import jax
import jax.numpy as jnp

def _softmax(x, axis=-1):
    return jax.nn.softmax(x, axis=axis)
def _gelu(x):
    return jax.nn.gelu(x, approximate=True)
def _silu(x):
    return jax.nn.silu(x)
def _sigmoid(x):
    return jax.nn.sigmoid(x)
def _layernorm(x, axis=-1, eps=1e-5):
    m = jnp.mean(x, axis=axis, keepdims=True)
    v = jnp.var(x, axis=axis, keepdims=True)
    return (x - m) / jnp.sqrt(v + eps)
def _scatter_add(tgt, idx, src, axis=0):
    return tgt.at[idx].add(src)
def _segment_sum(src, seg, n):
    return jax.ops.segment_sum(src, seg, n)
class _Rng:
    def __init__(self, key):
        self._k = key
    def _next(self):
        self._k, sub = jax.random.split(self._k)
        return sub
    def normal(self, shape):
        return jax.random.normal(self._next(), shape, dtype=jnp.bfloat16)
    def randint(self, lo, hi, shape):
        return jax.random.randint(self._next(), shape, lo, hi, dtype=jnp.int32)
    def uniform(self, shape, lo=0.0, hi=1.0):
        return jax.random.uniform(self._next(), shape, jnp.bfloat16, lo, hi)
    def permutation(self, n):
        return jax.random.permutation(self._next(), n)


kernel_name = 'gated_mix__ssm_conv_s5__geglu_ffn__prompt'

def setup_inputs():
    _rng = _Rng(jax.random.key(int.from_bytes(__import__("os").urandom(4), "little")))
    _w = (lambda a: (lambda t: t.astype(jnp.bfloat16) if jnp.issubdtype(t.dtype, jnp.floating) else t)(jnp.asarray(a)))
    def _A_setup():
        B, S, D = 1, 2048, 512
        P = D
        Lambda_re = -0.5 * jnp.exp((lambda *s: _rng.normal(s) * 0.4)(P))
        Lambda_im = (lambda *s: _rng.normal(s) * 0.4)(P) * 1.0
        B_re = (lambda *s: _rng.normal(s) * 0.4)(P, D) * (D ** -0.5)
        B_im = (lambda *s: _rng.normal(s) * 0.4)(P, D) * (D ** -0.5)
        C_re = (lambda *s: _rng.normal(s) * 0.4)(D, P) * (P ** -0.5)
        C_im = (lambda *s: _rng.normal(s) * 0.4)(D, P) * (P ** -0.5)
        log_dt = (lambda *s: _rng.normal(s) * 0.4)(P) * 0.3 - 2.0
        Dskip = (lambda *s: _rng.normal(s) * 0.4)(D)
        return {
            "x": _w((lambda *s: _rng.normal(s) * 0.05)(B, S, D)),
            "Lambda_re": _w(Lambda_re),
            "Lambda_im": _w(Lambda_im),
            "B_re": _w(B_re),
            "B_im": _w(B_im),
            "C_re": _w(C_re),
            "C_im": _w(C_im),
            "log_dt": _w(log_dt),
            "Dskip": _w(Dskip),
        }
    _A_in = _A_setup()

    def _B_setup():
        B, S, D, F = 1, 2048, 512, 1376
        return {
            "x": _w((lambda *s: _rng.normal(s) * 0.05)(B, S, D)),
            "w_gate": _w((lambda *s: _rng.normal(s) * 0.1)(D, F)),
            "w_up": _w((lambda *s: _rng.normal(s) * 0.1)(D, F)),
            "w_down": _w((lambda *s: _rng.normal(s) * 0.1)(F, D)),
        }
    _B_in = _B_setup()

    return {
        "A_x": _A_in["x"],
        "A_Lambda_re": _A_in["Lambda_re"],
        "A_Lambda_im": _A_in["Lambda_im"],
        "A_B_re": _A_in["B_re"],
        "A_B_im": _A_in["B_im"],
        "A_C_re": _A_in["C_re"],
        "A_C_im": _A_in["C_im"],
        "A_log_dt": _A_in["log_dt"],
        "A_Dskip": _A_in["Dskip"],
        "B_x": _B_in["x"],
        "B_w_gate": _B_in["w_gate"],
        "B_w_up": _B_in["w_up"],
        "B_w_down": _B_in["w_down"],
        "gate_w": _w((lambda *s: _rng.normal(s) * 0.05)(512) * 16.0),
    }

def reference(A_x, A_Lambda_re, A_Lambda_im, A_B_re, A_B_im, A_C_re, A_C_im, A_log_dt, A_Dskip, B_x, B_w_gate, B_w_up, B_w_down, gate_w):
    def _A_ref(x, Lambda_re, Lambda_im, B_re, B_im, C_re, C_im, log_dt, Dskip):
        Bsz, L, H = x.shape
        Lam = Lambda_re + 1j * Lambda_im
        Bmat = B_re + 1j * B_im
        Cmat = C_re + 1j * C_im
        dt = jnp.exp(log_dt)
        Lam_bar = jnp.exp(dt * Lam)
        B_bar = ((Lam_bar - 1.0) / Lam)[:, None] * Bmat
        Bu = jnp.einsum("bld,pd->blp", x + 0j, B_bar)
        h = jnp.zeros_like(Bu[:, 0, :])
        hs = []
        for t in range(L):
            h = Lam_bar[None, :] * h + Bu[:, t, :]
            hs.append(h)
        hseq = jnp.stack(hs, 1)
        y = 2.0 * jnp.einsum("blp,dp->bld", hseq, Cmat).real + x * Dskip[None, None, :]
        return y

    def _B_ref(x, w_gate, w_up, w_down):
        return (_gelu(x @ w_gate) * (x @ w_up)) @ w_down

    x = A_x
    g = _sigmoid((x * gate_w).sum(-1, keepdims=True))
    a = _A_ref(x, A_Lambda_re, A_Lambda_im, A_B_re, A_B_im, A_C_re, A_C_im, A_log_dt, A_Dskip)
    b = _B_ref(x, B_w_gate, B_w_up, B_w_down)
    return g * a + (1 - g) * b
```

```python
import jax
import jax.numpy as jnp
from jax import lax
import jax.experimental.pallas as pl
import jax.experimental.pallas.tpu as pltpu

F32 = jnp.float32
BF16 = jnp.bfloat16

TB = 128
NC = 8
CL = TB // NC + 1
LAST = TB - (NC - 1) * CL
TBP = NC * CL


def _cmul(ar, ai, br, bi):
    return ar * br - ai * bi, ar * bi + ai * br


def _cpow(r, i, n):
    res = None
    while n:
        if n & 1:
            res = (r, i) if res is None else _cmul(res[0], res[1], r, i)
        n >>= 1
        if n:
            r, i = _cmul(r, i, r, i)
    return res


def _kernel(x_ref, lre_ref, lim_ref, bre_hbm, bim_hbm, cre_hbm, cim_hbm, ldt_ref,
            dskip_ref, wgt_hbm, wut_hbm, wd_hbm, gw_ref, o_ref,
            bcat_ref, ccat_ref, wgt_ref, wut_ref, wd_ref, sems,
            lam_ref, carry_ref, bu_ref, h_ref):
    P = lre_ref.shape[-1]
    NJ = 2 * P // 128
    step = pl.program_id(0)

    copies = [
        pltpu.make_async_copy(bre_hbm, bcat_ref.at[0:P, :], sems.at[0]),
        pltpu.make_async_copy(bim_hbm, bcat_ref.at[P:2 * P, :], sems.at[1]),
        pltpu.make_async_copy(wgt_hbm, wgt_ref, sems.at[2]),
        pltpu.make_async_copy(wut_hbm, wut_ref, sems.at[3]),
        pltpu.make_async_copy(cre_hbm, ccat_ref.at[:, 0:P], sems.at[4]),
        pltpu.make_async_copy(cim_hbm, ccat_ref.at[:, P:2 * P], sems.at[5]),
        pltpu.make_async_copy(wd_hbm, wd_ref, sems.at[6]),
    ]

    @pl.when(step == 0)
    def _init():
        for c in copies:
            c.start()
        lre = lre_ref[...].reshape(1, P).astype(F32)
        lim = lim_ref[...].reshape(1, P).astype(F32)
        dt = jnp.exp(ldt_ref[...].reshape(1, P).astype(F32)).astype(BF16).astype(F32)
        mag = jnp.exp(dt * lre)
        ang = dt * lim
        lbr = mag * jnp.cos(ang)
        lbi = mag * jnp.sin(ang)
        nr = lbr - 1.0
        ni = lbi
        den = lre * lre + lim * lim
        cr = (nr * lre + ni * lim) / den
        ci = (ni * lre - nr * lim) / den
        pr, pi = _cpow(lbr, lbi, CL)
        lam_ref[0:1, :] = lbr
        lam_ref[1:2, :] = lbi
        lam_ref[2:3, :] = pr
        lam_ref[3:4, :] = pi
        lam_ref[4:5, :] = cr
        lam_ref[5:6, :] = ci
        lam_ref[6:8, :] = jnp.zeros((2, P), F32)
        carry_ref[...] = jnp.zeros_like(carry_ref)
        bu_ref[:, TB:TBP, :] = jnp.zeros((NJ, TBP - TB, 128), F32)

    nt = (((1,), (1,)), ((), ()))

    def body(first):
        def wait(*idx):
            if first:
                for k in idx:
                    copies[k].wait()

        x = x_ref[...]
        wait(0, 1)
        uv = lax.dot_general(x, bcat_ref[...], nt, preferred_element_type=F32)
        cr = lam_ref[4:5, :]
        ci = lam_ref[5:6, :]
        u = uv[:, 0:P]
        v = uv[:, P:2 * P]
        bur = cr * u - ci * v
        bui = cr * v + ci * u
        for j in range(NJ // 2):
            bu_ref[j, 0:TB, :] = bur[:, j * 128:(j + 1) * 128]
            bu_ref[NJ // 2 + j, 0:TB, :] = bui[:, j * 128:(j + 1) * 128]

        wait(2)
        gate = lax.dot_general(x, wgt_ref[...], nt, preferred_element_type=F32)

        def ld(ref, t, j0):
            return jnp.concatenate(
                [ref[j0 + j, pl.ds(t, NC, stride=CL), :] for j in range(NJ // 2)], axis=1)

        def st(ref, t, j0, v):
            for j in range(NJ // 2):
                ref[j0 + j, pl.ds(t, NC, stride=CL), :] = v[:, j * 128:(j + 1) * 128]

        sub = lax.broadcasted_iota(jnp.int32, (NC, P), 0)
        lr = jnp.broadcast_to(lam_ref[0:1, :], (NC, P))
        li = jnp.broadcast_to(lam_ref[1:2, :], (NC, P))
        lr2 = jnp.where(sub == NC - 1, 1.0, lr)
        li2 = jnp.where(sub == NC - 1, 0.0, li)
        ar = lam_ref[2:3, :]
        ai = lam_ref[3:4, :]

        def rec(hr, hi, t):
            br = ld(bu_ref, t, 0)
            bi = ld(bu_ref, t, NJ // 2)
            mr, mi = (lr, li) if t < LAST else (lr2, li2)
            return mr * hr - mi * hi + br, mr * hi + mi * hr + bi

        hr = ld(bu_ref, 0, 0)
        hi = ld(bu_ref, 0, NJ // 2)
        for t in range(1, CL):
            hr, hi = rec(hr, hi, t)

        er = carry_ref[0:1, :]
        ei = carry_ref[1:2, :]
        ir = jnp.zeros((NC, P), F32)
        ii = jnp.zeros((NC, P), F32)
        for c in range(NC):
            ir = jnp.where(sub == c, jnp.broadcast_to(er, (NC, P)), ir)
            ii = jnp.where(sub == c, jnp.broadcast_to(ei, (NC, P)), ii)
            if c < NC - 1:
                tr, ti = _cmul(ar, ai, er, ei)
                er = hr[c:c + 1, :] + tr
                ei = hi[c:c + 1, :] + ti

        hr, hi = ir, ii
        for t in range(CL):
            hr, hi = rec(hr, hi, t)
            st(h_ref, t, 0, hr)
            st(h_ref, t, NJ // 2, -hi)
        carry_ref[0:1, :] = hr[NC - 1:NC, :]
        carry_ref[1:2, :] = hi[NC - 1:NC, :]

        wait(3)
        up = lax.dot_general(x, wut_ref[...], nt, preferred_element_type=F32)
        act = (jax.nn.gelu(gate, approximate=True) * up).astype(BF16)

        wait(4, 5)
        hall = jnp.concatenate([h_ref[j, 0:TB, :] for j in range(NJ)], axis=1).astype(BF16)
        y = lax.dot_general(hall, ccat_ref[...], nt, preferred_element_type=F32)
        xf = x.astype(F32)
        a = 2.0 * y + xf * dskip_ref[...].reshape(1, P).astype(F32)

        wait(6)
        b = jnp.dot(act, wd_ref[...], preferred_element_type=F32)

        g = jax.nn.sigmoid(
            jnp.sum(xf * gw_ref[...].reshape(1, P).astype(F32), axis=-1, keepdims=True))
        o_ref[...] = g * a + (1.0 - g) * b


    @pl.when(step == 0)
    def _():
        body(True)

    @pl.when(step > 0)
    def _():
        body(False)


@jax.jit
def pallas_gated_mix__ssm_conv_s5__geglu_ffn__prompt_kernel(
    A_x: jax.Array,
    A_Lambda_re: jax.Array,
    A_Lambda_im: jax.Array,
    A_B_re: jax.Array,
    A_B_im: jax.Array,
    A_C_re: jax.Array,
    A_C_im: jax.Array,
    A_log_dt: jax.Array,
    A_Dskip: jax.Array,
    B_x: jax.Array,
    B_w_gate: jax.Array,
    B_w_up: jax.Array,
    B_w_down: jax.Array,
    gate_w: jax.Array,
):
    Bsz, L, D = A_x.shape
    P = A_Lambda_re.shape[0]
    Fdim = B_w_gate.shape[1]
    assert Bsz == 1 and L % TB == 0
    x2 = A_x.reshape(L, D)

    vec = pl.BlockSpec((P,), lambda i: (0,))
    hbm = pl.BlockSpec(memory_space=pl.ANY)

    out = pl.pallas_call(
        _kernel,
        grid=(L // TB,),
        in_specs=[
            pl.BlockSpec((TB, D), lambda i: (i, 0)),
            vec, vec,
            hbm, hbm, hbm, hbm,
            vec, vec,
            hbm, hbm, hbm,
            vec,
        ],
        out_specs=pl.BlockSpec((TB, D), lambda i: (i, 0)),
        out_shape=jax.ShapeDtypeStruct((L, D), F32),
        scratch_shapes=[
            pltpu.VMEM((2 * P, D), BF16),
            pltpu.VMEM((D, 2 * P), BF16),
            pltpu.VMEM((Fdim, D), BF16),
            pltpu.VMEM((Fdim, D), BF16),
            pltpu.VMEM((Fdim, D), BF16),
            pltpu.SemaphoreType.DMA((7,)),
            pltpu.VMEM((8, P), F32),
            pltpu.VMEM((8, P), F32),
            pltpu.VMEM((2 * P // 128, TBP, 128), F32),
            pltpu.VMEM((2 * P // 128, TBP, 128), F32),
        ],
        compiler_params=pltpu.CompilerParams(
            dimension_semantics=("arbitrary",),
            vmem_limit_bytes=64 * 1024 * 1024,
        ),
    )(x2, A_Lambda_re, A_Lambda_im, A_B_re, A_B_im,
      A_C_re, A_C_im, A_log_dt, A_Dskip,
      B_w_gate.T, B_w_up.T, B_w_down, gate_w)
    return out.reshape(Bsz, L, D)
```

```python
import jax
import jax.numpy as jnp
from jax import lax
import jax.experimental.pallas as pl
import jax.experimental.pallas.tpu as pltpu

F32 = jnp.float32
BF16 = jnp.bfloat16

TB = 256
NC = 8
CL = TB // NC + 1
LAST = TB - (NC - 1) * CL
TBP = NC * CL


def _cmul(ar, ai, br, bi):
    return ar * br - ai * bi, ar * bi + ai * br


def _cpow(r, i, n):
    res = None
    while n:
        if n & 1:
            res = (r, i) if res is None else _cmul(res[0], res[1], r, i)
        n >>= 1
        if n:
            r, i = _cmul(r, i, r, i)
    return res


def _kernel(x_ref, lre_ref, lim_ref, bre_ref, bim_ref, cre_hbm, cim_hbm, ldt_ref,
            dskip_ref, wgt_hbm, wut_hbm, wd_hbm, gw_ref, o_ref,
            ccat_ref, wgt_ref, wut_ref, wd_ref, sems,
            lam_ref, carry_ref, bu_ref, h_ref):
    P = lre_ref.shape[-1]
    NJ = 2 * P // 128
    step = pl.program_id(0)

    copies = [
        pltpu.make_async_copy(wgt_hbm, wgt_ref, sems.at[0]),
        pltpu.make_async_copy(wut_hbm, wut_ref, sems.at[1]),
        pltpu.make_async_copy(cre_hbm, ccat_ref.at[:, 0:P], sems.at[2]),
        pltpu.make_async_copy(cim_hbm, ccat_ref.at[:, P:2 * P], sems.at[3]),
        pltpu.make_async_copy(wd_hbm, wd_ref, sems.at[4]),
    ]

    @pl.when(step == 0)
    def _init():
        for c in copies:
            c.start()
        lre = lre_ref[...].reshape(1, P).astype(F32)
        lim = lim_ref[...].reshape(1, P).astype(F32)
        dt = jnp.exp(ldt_ref[...].reshape(1, P).astype(F32)).astype(BF16).astype(F32)
        mag = jnp.exp(dt * lre)
        ang = dt * lim
        lbr = mag * jnp.cos(ang)
        lbi = mag * jnp.sin(ang)
        nr = lbr - 1.0
        ni = lbi
        den = lre * lre + lim * lim
        cr = (nr * lre + ni * lim) / den
        ci = (ni * lre - nr * lim) / den
        pr, pi = _cpow(lbr, lbi, CL)
        lam_ref[0:1, :] = lbr
        lam_ref[1:2, :] = lbi
        lam_ref[2:3, :] = pr
        lam_ref[3:4, :] = pi
        lam_ref[4:5, :] = cr
        lam_ref[5:6, :] = ci
        lam_ref[6:8, :] = jnp.zeros((2, P), F32)
        carry_ref[...] = jnp.zeros_like(carry_ref)
        bu_ref[:, TB:TBP, :] = jnp.zeros((NJ, TBP - TB, 128), F32)

    nt = (((1,), (1,)), ((), ()))

    def body(first):
        def wait(*idx):
            if first:
                for k in idx:
                    copies[k].wait()

        x = x_ref[...]
        u = lax.dot_general(x, bre_ref[...], nt, preferred_element_type=F32)
        v = lax.dot_general(x, bim_ref[...], nt, preferred_element_type=F32)
        cr = lam_ref[4:5, :]
        ci = lam_ref[5:6, :]
        bur = cr * u - ci * v
        bui = cr * v + ci * u
        for j in range(NJ // 2):
            bu_ref[j, 0:TB, :] = bur[:, j * 128:(j + 1) * 128]
            bu_ref[NJ // 2 + j, 0:TB, :] = bui[:, j * 128:(j + 1) * 128]

        wait(0)
        gate = lax.dot_general(x, wgt_ref[...], nt, preferred_element_type=F32)

        def ld(ref, t, j0):
            return jnp.concatenate(
                [ref[j0 + j, pl.ds(t, NC, stride=CL), :] for j in range(NJ // 2)], axis=1)

        def st(ref, t, j0, v):
            for j in range(NJ // 2):
                ref[j0 + j, pl.ds(t, NC, stride=CL), :] = v[:, j * 128:(j + 1) * 128]

        sub = lax.broadcasted_iota(jnp.int32, (NC, P), 0)
        lr = jnp.broadcast_to(lam_ref[0:1, :], (NC, P))
        li = jnp.broadcast_to(lam_ref[1:2, :], (NC, P))
        lr2 = jnp.where(sub == NC - 1, 1.0, lr)
        li2 = jnp.where(sub == NC - 1, 0.0, li)
        ar = lam_ref[2:3, :]
        ai = lam_ref[3:4, :]

        def rec(hr, hi, t):
            br = ld(bu_ref, t, 0)
            bi = ld(bu_ref, t, NJ // 2)
            mr, mi = (lr, li) if t < LAST else (lr2, li2)
            return mr * hr - mi * hi + br, mr * hi + mi * hr + bi

        hr = ld(bu_ref, 0, 0)
        hi = ld(bu_ref, 0, NJ // 2)
        for t in range(1, CL):
            hr, hi = rec(hr, hi, t)

        er = carry_ref[0:1, :]
        ei = carry_ref[1:2, :]
        ir = jnp.zeros((NC, P), F32)
        ii = jnp.zeros((NC, P), F32)
        for c in range(NC):
            ir = jnp.where(sub == c, jnp.broadcast_to(er, (NC, P)), ir)
            ii = jnp.where(sub == c, jnp.broadcast_to(ei, (NC, P)), ii)
            if c < NC - 1:
                tr, ti = _cmul(ar, ai, er, ei)
                er = hr[c:c + 1, :] + tr
                ei = hi[c:c + 1, :] + ti

        hr, hi = ir, ii
        for t in range(CL):
            hr, hi = rec(hr, hi, t)
            st(h_ref, t, 0, hr)
            st(h_ref, t, NJ // 2, -hi)
        carry_ref[0:1, :] = hr[NC - 1:NC, :]
        carry_ref[1:2, :] = hi[NC - 1:NC, :]

        wait(1)
        up = lax.dot_general(x, wut_ref[...], nt, preferred_element_type=F32)
        act = (jax.nn.gelu(gate, approximate=True) * up).astype(BF16)

        wait(2, 3)
        hall = jnp.concatenate([h_ref[j, 0:TB, :] for j in range(NJ)], axis=1).astype(BF16)
        y = lax.dot_general(hall, ccat_ref[...], nt, preferred_element_type=F32)
        xf = x.astype(F32)
        a = 2.0 * y + xf * dskip_ref[...].reshape(1, P).astype(F32)

        wait(4)
        b = jnp.dot(act, wd_ref[...], preferred_element_type=F32)

        g = jax.nn.sigmoid(
            jnp.sum(xf * gw_ref[...].reshape(1, P).astype(F32), axis=-1, keepdims=True))
        o_ref[...] = g * a + (1.0 - g) * b


    @pl.when(step == 0)
    def _():
        body(True)

    @pl.when(step > 0)
    def _():
        body(False)


@jax.jit
def pallas_gated_mix__ssm_conv_s5__geglu_ffn__prompt_kernel(
    A_x: jax.Array,
    A_Lambda_re: jax.Array,
    A_Lambda_im: jax.Array,
    A_B_re: jax.Array,
    A_B_im: jax.Array,
    A_C_re: jax.Array,
    A_C_im: jax.Array,
    A_log_dt: jax.Array,
    A_Dskip: jax.Array,
    B_x: jax.Array,
    B_w_gate: jax.Array,
    B_w_up: jax.Array,
    B_w_down: jax.Array,
    gate_w: jax.Array,
):
    Bsz, L, D = A_x.shape
    P = A_Lambda_re.shape[0]
    Fdim = B_w_gate.shape[1]
    assert Bsz == 1 and L % TB == 0
    x2 = A_x.reshape(L, D)

    vec = pl.BlockSpec((P,), lambda i: (0,))
    hbm = pl.BlockSpec(memory_space=pl.ANY)

    out = pl.pallas_call(
        _kernel,
        grid=(L // TB,),
        in_specs=[
            pl.BlockSpec((TB, D), lambda i: (i, 0)),
            vec, vec,
            pl.BlockSpec((P, D), lambda i: (0, 0)), pl.BlockSpec((P, D), lambda i: (0, 0)), hbm, hbm,
            vec, vec,
            hbm, hbm, hbm,
            vec,
        ],
        out_specs=pl.BlockSpec((TB, D), lambda i: (i, 0)),
        out_shape=jax.ShapeDtypeStruct((L, D), F32),
        scratch_shapes=[
            pltpu.VMEM((D, 2 * P), BF16),
            pltpu.VMEM((Fdim, D), BF16),
            pltpu.VMEM((Fdim, D), BF16),
            pltpu.VMEM((Fdim, D), BF16),
            pltpu.SemaphoreType.DMA((5,)),
            pltpu.VMEM((8, P), F32),
            pltpu.VMEM((8, P), F32),
            pltpu.VMEM((2 * P // 128, TBP, 128), F32),
            pltpu.VMEM((2 * P // 128, TBP, 128), F32),
        ],
        compiler_params=pltpu.CompilerParams(
            dimension_semantics=("arbitrary",),
            vmem_limit_bytes=64 * 1024 * 1024,
        ),
    )(x2, A_Lambda_re, A_Lambda_im, A_B_re, A_B_im,
      A_C_re, A_C_im, A_log_dt, A_Dskip,
      B_w_gate.T, B_w_up.T, B_w_down, gate_w)
    return out.reshape(Bsz, L, D)
```
